```python
import os as _os
_os.environ.setdefault("JAX_PLATFORMS", "cpu")
import jax
import jax.numpy as jnp

def _softmax(x, axis=-1):
    return jax.nn.softmax(x, axis=axis)
def _gelu(x):
    return jax.nn.gelu(x, approximate=True)
def _silu(x):
    return jax.nn.silu(x)
def _sigmoid(x):
    return jax.nn.sigmoid(x)
def _layernorm(x, axis=-1, eps=1e-5):
    m = jnp.mean(x, axis=axis, keepdims=True)
    v = jnp.var(x, axis=axis, keepdims=True)
    return (x - m) / jnp.sqrt(v + eps)
def _scatter_add(tgt, idx, src, axis=0):
    return tgt.at[idx].add(src)
def _segment_sum(src, seg, n):
    return jax.ops.segment_sum(src, seg, n)
class _Rng:
    def __init__(self, key):
        self._k = key
    def _next(self):
        self._k, sub = jax.random.split(self._k)
        return sub
    def normal(self, shape):
        return jax.random.normal(self._next(), shape, dtype=jnp.bfloat16)
    def randint(self, lo, hi, shape):
        return jax.random.randint(self._next(), shape, lo, hi, dtype=jnp.int32)
    def uniform(self, shape, lo=0.0, hi=1.0):
        return jax.random.uniform(self._next(), shape, jnp.bfloat16, lo, hi)
    def permutation(self, n):
        return jax.random.permutation(self._next(), n)


kernel_name = 'parallel_sum__mha_block__swiglu_ffn__prompt'

def setup_inputs():
    _rng = _Rng(jax.random.key(int.from_bytes(__import__("os").urandom(4), "little")))
    _w = (lambda a: (lambda t: t.astype(jnp.bfloat16) if jnp.issubdtype(t.dtype, jnp.floating) else t)(jnp.asarray(a)))
    def _A_setup():
        B, S, D, H = 1, 2048, 512, 32
        return {
            "x": _w((lambda *s: _rng.normal(s) * 0.05)(B, S, D)),
            "wqkv": _w((lambda *s: _rng.normal(s) * 0.1)(D, 3 * D)),
            "wo": _w((lambda *s: _rng.normal(s) * 0.05)(D, D)),
        }
    _A_in = _A_setup()

    def _B_setup():
        B, S, D, F = 1, 2048, 512, 1792
        return {
            "x": _w((lambda *s: _rng.normal(s) * 0.05)(B, S, D)),
            "w_gate": _w((lambda *s: _rng.normal(s) * 0.05)(D, F)),
            "w_up": _w((lambda *s: _rng.normal(s) * 0.05)(D, F)),
            "w_down": _w((lambda *s: _rng.normal(s) * 0.05)(F, D)),
        }
    _B_in = _B_setup()

    return {
        "A_x": _A_in["x"],
        "A_wqkv": _A_in["wqkv"],
        "A_wo": _A_in["wo"],
        "B_x": _B_in["x"],
        "B_w_gate": _B_in["w_gate"],
        "B_w_up": _B_in["w_up"],
        "B_w_down": _B_in["w_down"],
    }

def reference(A_x, A_wqkv, A_wo, B_x, B_w_gate, B_w_up, B_w_down):
    def _A_ref(x, wqkv, wo):
        B, S, D = x.shape
        H = 32
        Dh = D // H
        qkv = (lambda x, *d: x.transpose(*d))((x @ wqkv).reshape(B, S, 3, H, Dh), 2, 0, 3, 1, 4)
        q, k, v = qkv[0], qkv[1], qkv[2]
        scores = jnp.einsum("bhqd,bhkd->bhqk", q, k) * (Dh ** -0.5)
        p = _softmax(scores, axis=-1)
        o = jnp.einsum("bhqk,bhkd->bhqd", p, v)
        return (lambda x, *d: x.transpose(*d))(o, 0, 2, 1, 3).reshape(B, S, D) @ wo

    def _B_ref(x, w_gate, w_up, w_down):
        g = _silu(x @ w_gate)
        u = x @ w_up
        return (g * u) @ w_down

    x = A_x
    xn = _layernorm(x, axis=-1)
    return x + _A_ref(xn, A_wqkv, A_wo) + _B_ref(xn, B_w_gate, B_w_up, B_w_down)
```

```python
import functools

import jax
import jax.numpy as jnp
import jax.experimental.pallas as pl
import jax.experimental.pallas.tpu as pltpu

H = 32
LOG2E = 1.4426950408889634


def _kernel(x_ref, wqkv_ref, wo_hbm, wg_hbm, wu_hbm, wd_hbm, o_ref,
            xn_ref, k_ref, qt_ref, vt_ref, ot_ref, s_ref, m_ref, l_ref, w_ref, wo_ref, wg_ref, wu_ref, wd_ref, sem, *, S, D, QB, HU, CH):
    Dh = D // H
    G = D // 128
    HPG = 128 // Dh
    NB = S // QB
    i = pl.program_id(0)
    f32 = jnp.float32
    bf16 = jnp.bfloat16

    copies = [pltpu.make_async_copy(src, dst, sem.at[n]) for n, (src, dst) in enumerate(
        ((wg_hbm, wg_ref), (wu_hbm, wu_ref), (wd_hbm, wd_ref), (wo_hbm, wo_ref)))]

    @pl.when(i == 0)
    def _prologue():
        for cp in copies:
            cp.start()
        for b in range(NB):
            rows = pl.ds(b * QB, QB)
            x = x_ref[rows, :].astype(f32)
            m = jnp.mean(x, axis=-1, keepdims=True)
            xc = x - m
            v = jnp.mean(xc * xc, axis=-1, keepdims=True)
            xn = (xc * jax.lax.rsqrt(v + 1e-5)).astype(bf16)
            xn_ref[rows, :] = xn
            q = jnp.dot(xn, wqkv_ref[:, 0:D], preferred_element_type=f32)
            q = q * (Dh ** -0.5 * LOG2E)
            qt = q.T.astype(bf16)
            k = jnp.dot(xn, wqkv_ref[:, D:2 * D], preferred_element_type=f32).astype(bf16)
            vv = jnp.dot(xn, wqkv_ref[:, 2 * D:3 * D], preferred_element_type=f32)
            vt = vv.T.astype(bf16)
            for g in range(G):
                qt_ref[b, g] = qt[g * 128:(g + 1) * 128, :]
                k_ref[g, rows, :] = k[:, g * 128:(g + 1) * 128]
            vt_ref[:, :, b * QB:(b + 1) * QB] = vt.reshape(H, Dh, QB)

    row_head = jax.lax.broadcasted_iota(jnp.int32, (128, QB), 0) // Dh
    NC = S // CH

    def qk_weights(b, h):
        return jnp.where(row_head == h % HPG, qt_ref[b, h // HPG], jnp.zeros((), bf16))

    def qk_chunk(w, g, slot, c, m):
        rows = pl.ds(c * CH, CH)
        st = jnp.dot(k_ref[g, rows, :], w, preferred_element_type=f32)
        s_ref[slot, rows, :] = st
        cm = jnp.max(st.reshape(CH // 8, 8, QB), axis=0)
        return cm if m is None else jnp.maximum(m, cm)

    def fin_max(m):
        return jnp.max(m, axis=0, keepdims=True)

    @pl.when(i == 0)
    def _first():
        w = qk_weights(0, 0)
        m = None
        for c in range(NC):
            m = qk_chunk(w, 0, 0, c, m)
        m_ref[...] = jnp.broadcast_to(fin_max(m), (8, QB))
        w_ref[0] = qk_weights(0, 1)

    def step(h, slot):
        if True:
            nh = (h + 1) % H
            w = w_ref[slot]
            mcur = m_ref[0:1, :]
            m = None
            acc = None
            for c in range(NC):
                rows = pl.ds(c * CH, CH)
                p = jnp.exp2(s_ref[slot, rows, :] - mcur)
                lc = jnp.sum(p.reshape(CH // 8, 8, QB), axis=0)
                if c == 0:
                    l_ref[...] = lc
                else:
                    l_ref[...] += lc
                pv = jnp.dot(vt_ref[h, :, c * CH:(c + 1) * CH], p.astype(bf16),
                             preferred_element_type=f32)
                acc = pv if acc is None else acc + pv
                m = qk_chunk(w, nh // HPG, 1 - slot, c, m)
            w_ref[1 - slot] = qk_weights(jnp.minimum(i + (h + 2) // H, NB - 1), (h + 2) % H)
            ot_ref[h] = acc * (1.0 / jnp.sum(l_ref[...], axis=0, keepdims=True))
            m_ref[...] = jnp.broadcast_to(fin_max(m), (8, QB))

    def body(h, carry):
        pl.when(h % 2 == 0)(lambda: step(h, 0))
        pl.when(h % 2 == 1)(lambda: step(h, 1))
        return carry

    jax.lax.fori_loop(0, H, body, 0)

    rows = pl.ds(pl.multiple_of(i * QB, QB), QB)

    @pl.when(i == 0)
    def _():
        for cp in copies:
            cp.wait()

    xn = xn_ref[rows, :]
    gt = jnp.dot(xn, wg_ref[...], preferred_element_type=f32)
    up = jnp.dot(xn, wu_ref[...], preferred_element_type=f32)
    hmid = (gt * jax.nn.sigmoid(gt) * up).astype(bf16)
    ffn = jnp.dot(hmid, wd_ref[...], preferred_element_type=f32)
    o = ot_ref[...].reshape(D, QB).T.astype(bf16)
    att = jnp.dot(o, wo_ref[...], preferred_element_type=f32)
    o_ref[...] = (x_ref[rows, :].astype(f32) + att + ffn).astype(o_ref.dtype)


@jax.jit
def pallas_parallel_sum__mha_block__swiglu_ffn__prompt_kernel(
    A_x: jax.Array,
    A_wqkv: jax.Array,
    A_wo: jax.Array,
    B_x: jax.Array,
    B_w_gate: jax.Array,
    B_w_up: jax.Array,
    B_w_down: jax.Array,
):
    del B_x
    B, S, D = A_x.shape
    F = B_w_gate.shape[1]
    QB, HU, CH = 512, 2, 128
    Dh = D // H
    x = A_x.reshape(S, D)
    full = lambda a: pl.BlockSpec(a.shape, lambda i: (0,) * a.ndim)
    any_ = pl.BlockSpec(memory_space=pl.ANY)
    out = pl.pallas_call(
        functools.partial(_kernel, S=S, D=D, QB=QB, HU=HU, CH=CH),
        grid=(S // QB,),
        in_specs=[full(x), full(A_wqkv), any_, any_, any_, any_],
        out_specs=pl.BlockSpec((QB, D), lambda i: (i, 0)),
        out_shape=jax.ShapeDtypeStruct((S, D), A_x.dtype),
        scratch_shapes=[
            pltpu.VMEM((S, D), jnp.bfloat16),
            pltpu.VMEM((D // 128, S, 128), jnp.bfloat16),
            pltpu.VMEM((S // QB, D // 128, 128, QB), jnp.bfloat16),
            pltpu.VMEM((H, Dh, S), jnp.bfloat16),
            pltpu.VMEM((H, Dh, QB), jnp.float32),
            pltpu.VMEM((2, S, QB), jnp.float32),
            pltpu.VMEM((8, QB), jnp.float32),
            pltpu.VMEM((8, QB), jnp.float32),
            pltpu.VMEM((2, 128, QB), jnp.bfloat16),
            pltpu.VMEM((D, D), jnp.bfloat16),
            pltpu.VMEM((D, F), jnp.bfloat16),
            pltpu.VMEM((D, F), jnp.bfloat16),
            pltpu.VMEM((F, D), jnp.bfloat16),
            pltpu.SemaphoreType.DMA((4,)),
        ],
        compiler_params=pltpu.CompilerParams(
            dimension_semantics=("arbitrary",),
            vmem_limit_bytes=100 * 1024 * 1024,
        ),
    )(x, A_wqkv, A_wo, B_w_gate, B_w_up, B_w_down)
    return out.reshape(B, S, D)
```
